```python
import jax
import jax.numpy as jnp

def _softmax(x, axis=-1):
    return jax.nn.softmax(x, axis=axis)

def _gelu(x):
    return jax.nn.gelu(x, approximate=True)

def _silu(x):
    return jax.nn.silu(x)

def _sigmoid(x):
    return jax.nn.sigmoid(x)

def _layernorm(x, axis=-1, eps=1e-05):
    m = jnp.mean(x, axis=axis, keepdims=True)
    v = jnp.var(x, axis=axis, keepdims=True)
    return (x - m) / jnp.sqrt(v + eps)

def _scatter_add(tgt, idx, src, axis=0):
    return tgt.at[idx].add(src)

def _segment_sum(src, seg, n):
    return jax.ops.segment_sum(src, seg, n)

class _Rng:

    def __init__(self, key):
        self._k = key

    def _next(self):
        self._k, sub = jax.random.split(self._k)
        return sub

    def normal(self, shape):
        return jax.random.normal(self._next(), shape, dtype=jnp.bfloat16)

    def randint(self, lo, hi, shape):
        return jax.random.randint(self._next(), shape, lo, hi, dtype=jnp.int32)

    def uniform(self, shape, lo=0.0, hi=1.0):
        return jax.random.uniform(self._next(), shape, jnp.bfloat16, lo, hi)

    def permutation(self, n):
        return jax.random.permutation(self._next(), n)
kernel_name = 'recurrent_scan__memory_aug_recurrent_mem_tr__glu_gated_glu__prompt'

def setup_inputs():
    _rng = _Rng(jax.random.key(int.from_bytes(__import__("os").urandom(4), "little")))
    _w = lambda a: (lambda t: t.astype(jnp.bfloat16) if jnp.issubdtype(t.dtype, jnp.floating) else t)(jnp.asarray(a))

    def _A_setup():
        B, S, Dm = (1, 2048, 1024)
        H, Dh = (32, 128)
        M, seg = (8, 32)
        seg = min(seg, S)
        S = S // seg * seg
        return {'x': _w((lambda *s: _rng.normal(s) * 0.05)(B, S, Dm)), 'mem0': _w((lambda *s: _rng.normal(s) * 0.05)(B, M, Dm)), 'Wq': _w((lambda *s: _rng.normal(s) * 0.05)(Dm, H, Dh) * Dm ** (-0.5)), 'Wk': _w((lambda *s: _rng.normal(s) * 0.05)(Dm, H, Dh) * Dm ** (-0.5)), 'Wv': _w((lambda *s: _rng.normal(s) * 0.05)(Dm, H, Dh) * Dm ** (-0.5)), 'Wo': _w((lambda *s: _rng.normal(s) * 0.05)(H, Dh, Dm) * (H * Dh) ** (-0.5)), 'seg_len': seg}
    _A_in = _A_setup()

    def _B_setup():
        B, S, D, F = (1, 2048, 1024, 3584)
        return {'x': _w((lambda *s: _rng.normal(s) * 0.05)(B, S, D)), 'w_gate': _w((lambda *s: _rng.normal(s) * 0.05)(D, F)), 'w_up': _w((lambda *s: _rng.normal(s) * 0.05)(D, F)), 'w_down': _w((lambda *s: _rng.normal(s) * 0.05)(F, D))}
    _B_in = _B_setup()
    return {'A_x': _A_in['x'], 'A_mem0': _A_in['mem0'], 'A_Wq': _A_in['Wq'], 'A_Wk': _A_in['Wk'], 'A_Wv': _A_in['Wv'], 'A_Wo': _A_in['Wo'], 'A_seg_len': _A_in['seg_len'], 'B_x': _B_in['x'], 'B_w_gate': _B_in['w_gate'], 'B_w_up': _B_in['w_up'], 'B_w_down': _B_in['w_down']}

def reference(A_x, A_mem0, A_Wq, A_Wk, A_Wv, A_Wo, A_seg_len, B_x, B_w_gate, B_w_up, B_w_down):

    def _A_ref(x, mem0, Wq, Wk, Wv, Wo, seg_len):
        B, S, Dm = x.shape
        H, Dh = (Wq.shape[1], Wq.shape[2])
        M = mem0.shape[1]
        scale = Dh ** (-0.5)
        n_seg = S // seg_len
        L = M + seg_len
        idx = jnp.arange(L)
        mask = (idx[:, None] < M) | (idx[:, None] >= idx[None, :])
        mem = mem0
        outs = []
        for s in range(n_seg):
            xs = x[:, s * seg_len:(s + 1) * seg_len, :].copy()
            h = jnp.concatenate([mem, xs], axis=1)
            q = jnp.einsum('btd,dhe->bhte', h, Wq)
            k = jnp.einsum('btd,dhe->bhte', h, Wk)
            v = jnp.einsum('btd,dhe->bhte', h, Wv)
            scores = jnp.einsum('bhqe,bhke->bhqk', q, k) * scale
            scores = jnp.where(mask[None, None], scores, -1000000000.0)
            p = _softmax(scores, axis=-1)
            o = jnp.einsum('bhqk,bhke->bhqe', p, v)
            o = jnp.einsum('bhte,hed->btd', o, Wo)
            mem = o[:, :M, :].copy()
            outs.append(o[:, M:, :])
        return jnp.concatenate(outs, axis=1)

    def _B_ref(x, w_gate, w_up, w_down):
        g = jnp.einsum('bsd,df->bsf', x, w_gate)
        u = jnp.einsum('bsd,df->bsf', x, w_up)
        h = _sigmoid(g) * u
        return jnp.einsum('bsf,fd->bsd', h, w_down)
    x = A_x
    xn = _layernorm(x, axis=-1)
    s = _A_ref(xn, A_mem0, A_Wq, A_Wk, A_Wv, A_Wo, A_seg_len)
    g = _silu(_B_ref(xn, B_w_gate, B_w_up, B_w_down))
    return x + s * g
```

```python
import functools
import jax
import jax.numpy as jnp
import numpy as np
from jax import lax
from jax.experimental import pallas as pl
from jax.experimental.pallas import tpu as pltpu

S, D, H, DH, M, SEG, F = 2048, 1024, 32, 128, 8, 32, 3584
L = M + SEG
NSEG = S // SEG
RB = 128
CPB = RB // SEG
FT = F // 128
FC = FT // CPB
KT = D // 128

f32 = jnp.float32
bf16 = jnp.bfloat16


def _mm(a, b):
    return lax.dot_general(a, b, (((1,), (0,)), ((), ())), preferred_element_type=f32)


def _mm_nt(a, b):
    return lax.dot_general(a, b, (((1,), (1,)), ((), ())), preferred_element_type=f32)


def _kernel(x_hbm, mem0_hbm, wq_hbm, wk_hbm, wv_hbm, wo_hbm, wg_hbm, wu_hbm, wd_hbm,
            out_hbm,
            x_v, xn_v, mem_v, wq_v, wk_v, wv_v, wo_v, wg_v, wu_v, wd_v,
            gacc_v, s_v, o_stage, sems, osem):
    cps = []
    def cp(src, dst, i):
        c = pltpu.make_async_copy(src, dst, sems.at[i])
        c.start()
        return c
    cx = cp(x_hbm, x_v, 0)
    cm = cp(mem0_hbm, mem_v, 1)
    cq = cp(wq_hbm, wq_v, 2)
    ck = cp(wk_hbm, wk_v, 3)
    cv = cp(wv_hbm, wv_v, 4)
    co = [cp(wo_hbm.at[:, pl.ds(n * 128, 128)], wo_v.at[n], 5) for n in range(KT)]
    cg = [cp(wg_hbm.at[:, pl.ds(n * 128, 128)], wg_v.at[n], 6) for n in range(FT)]
    cu = [cp(wu_hbm.at[:, pl.ds(n * 128, 128)], wu_v.at[n], 7) for n in range(FT)]
    cd = [cp(wd_hbm.at[:, pl.ds(n * 128, 128)], wd_v.at[n], 8) for n in range(KT)]

    cx.wait()
    def ln_body(i, _):
        r = pl.multiple_of(i * 64, 64)
        xx = x_v[pl.ds(r, 64), :].astype(f32)
        m = jnp.mean(xx, axis=-1, keepdims=True)
        xc = xx - m
        v = jnp.mean(xc * xc, axis=-1, keepdims=True)
        xn_v[pl.ds(r, 64), :] = xc / jnp.sqrt(v + 1e-5)
        return 0
    lax.fori_loop(0, S // 64, ln_body, 0)
    cm.wait(); cq.wait(); ck.wait(); cv.wait()
    for c in co + cg + cu + cd:
        c.wait()

    ri = lax.broadcasted_iota(jnp.int32, (L, L), 0)
    ci = lax.broadcasted_iota(jnp.int32, (L, L), 1)
    mask = (ri < M) | (ri >= ci)
    scale = DH ** -0.5

    def step(s, mem):
        r0 = pl.multiple_of(s * SEG, SEG)
        h = jnp.concatenate([mem, xn_v[pl.ds(r0, SEG), :]], axis=0)
        os_ = []
        for hd in range(H):
            q = _mm(h, wq_v[hd])
            k = _mm(h, wk_v[hd]).astype(bf16)
            v = _mm(h, wv_v[hd]).astype(bf16)
            sc = _mm_nt(q, k) * scale
            sc = jnp.where(mask, sc, -1e9)
            mx = jnp.max(sc, axis=-1, keepdims=True)
            e = jnp.exp(sc - mx)
            p = e / jnp.sum(e, axis=-1, keepdims=True)
            os_.append(_mm(p, v))
        cols = []
        for n in range(KT):
            acc = None
            for hd in range(H):
                t = _mm(os_[hd], wo_v[n, pl.ds(hd * 128, 128), :])
                acc = t if acc is None else acc + t
            cols.append(acc)
        o = jnp.concatenate(cols, axis=1)
        mem_next = o[:M].astype(bf16).astype(f32)
        sb = s % CPB
        s_v[pl.ds(pl.multiple_of(sb * SEG, SEG), SEG), :] = o[M:]

        b0 = pl.multiple_of((s // CPB) * RB, RB)
        xb = xn_v[pl.ds(b0, RB), :]
        hs = []
        for j in range(FC):
            g = _mm(xb, wg_v[sb * FC + j])
            u = _mm(xb, wu_v[sb * FC + j])
            hs.append((jax.nn.sigmoid(g) * u).astype(bf16))
        hh = jnp.concatenate(hs, axis=1)
        f0 = pl.multiple_of(sb * (FC * 128), 128)
        dn = jnp.concatenate([_mm(hh, wd_v[n, pl.ds(f0, FC * 128), :]) for n in range(KT)], axis=1)

        @pl.when(sb == 0)
        def _():
            gacc_v[...] = dn

        @pl.when(sb != 0)
        def _():
            gacc_v[...] += dn

        @pl.when(sb == CPB - 1)
        def _():
            b = s // CPB
            slot = b % 2
            @pl.when(b >= 2)
            def _():
                pltpu.make_async_copy(o_stage.at[slot], out_hbm.at[pl.ds(0, RB)], osem.at[slot]).wait()
            ga = gacc_v[...]
            gl = ga * jax.nn.sigmoid(ga)
            res = x_v[pl.ds(b0, RB), :].astype(f32) + s_v[...] * gl
            o_stage[slot] = res.astype(bf16)
            pltpu.make_async_copy(o_stage.at[slot], out_hbm.at[pl.ds(b0, RB)], osem.at[slot]).start()
        return mem_next

    lax.fori_loop(0, NSEG, step, mem_v[...].astype(f32))
    for slot in range(2):
        pltpu.make_async_copy(o_stage.at[slot], out_hbm.at[pl.ds(0, RB)], osem.at[slot]).wait()


@jax.jit
def pallas_recurrent_scan__memory_aug_recurrent_mem_tr__glu_gated_glu__prompt_kernel(
        A_x, A_mem0, A_Wq, A_Wk, A_Wv, A_Wo, A_seg_len, B_x, B_w_gate, B_w_up, B_w_down):
    x = A_x.reshape(S, D)
    mem0 = A_mem0.reshape(M, D)
    wq = jnp.transpose(A_Wq, (1, 0, 2))
    wk = jnp.transpose(A_Wk, (1, 0, 2))
    wv = jnp.transpose(A_Wv, (1, 0, 2))
    wo = A_Wo.reshape(H * DH, D)
    anyspec = pl.BlockSpec(memory_space=pl.ANY)
    out = pl.pallas_call(
        _kernel,
        out_shape=jax.ShapeDtypeStruct((S, D), bf16),
        in_specs=[anyspec] * 9,
        out_specs=anyspec,
        scratch_shapes=[
            pltpu.VMEM((S, D), bf16),
            pltpu.VMEM((S, D), f32),
            pltpu.VMEM((M, D), bf16),
            pltpu.VMEM((H, D, DH), bf16),
            pltpu.VMEM((H, D, DH), bf16),
            pltpu.VMEM((H, D, DH), bf16),
            pltpu.VMEM((KT, H * DH, 128), bf16),
            pltpu.VMEM((FT, D, 128), bf16),
            pltpu.VMEM((FT, D, 128), bf16),
            pltpu.VMEM((KT, F, 128), bf16),
            pltpu.VMEM((RB, D), f32),
            pltpu.VMEM((RB, D), f32),
            pltpu.VMEM((2, RB, D), bf16),
            pltpu.SemaphoreType.DMA((9,)),
            pltpu.SemaphoreType.DMA((2,)),
        ],
        compiler_params=pltpu.CompilerParams(vmem_limit_bytes=110 * 2**20),
    )(x, mem0, wq, wk, wv, wo, B_w_gate, B_w_up, B_w_down)
    return out.reshape(1, S, D)
```

```python
import functools
import jax
import jax.numpy as jnp
from jax import lax
from jax.experimental import pallas as pl
from jax.experimental.pallas import tpu as pltpu

S, D, H, DH, M, SEG, F = 2048, 1024, 32, 128, 8, 32, 3584
L = M + SEG
NSEG = S // SEG
KT = D // 128
FT = F // 128
CPB = 4
FC = FT // CPB
RB = 88
R = S - (NSEG // CPB) * RB
PB = 128
LNC = 64
NLN = (S - R) // LNC
RAW = 128
NRAW = 3 * D // RAW
LA = 3
NS = 4
ELAG = 4
LAG1, LAG2 = 1, 3
EPI_AT = 8

RG = 8

f32 = jnp.float32
bf16 = jnp.bfloat16
u32 = jnp.uint32


def _mm(a, b):
    return lax.dot_general(a, b, (((1,), (0,)), ((), ())), preferred_element_type=f32)


def _mm_nt(a, b):
    return lax.dot_general(a, b, (((1,), (1,)), ((), ())), preferred_element_type=f32)


def _ln(xx):
    m = jnp.mean(xx, axis=-1, keepdims=True)
    xc = xx - m
    v = jnp.mean(xc * xc, axis=-1, keepdims=True)
    return xc / jnp.sqrt(v + 1e-5)


def _kernel(x_hbm, mem0_hbm, wq_hbm, wk_hbm, wv_hbm, wo_hbm, wg_hbm, wu_hbm, wd_hbm,
            out_hbm,
            x_v, xn_v, mem_v, wall_v, wo_v,
            g_v, s_v, o_v, stage, sem0, semc, semr, semo, semw):
    w32, wo32 = wall_v.bitcast(u32), wo_v.bitcast(u32)
    GO, UO = 3 * H, 3 * H + FT
    DO = (3 * H + 2 * FT) * D

    def WS(r0, n):
        if isinstance(r0, int):
            return pltpu.bitcast(w32[r0 // 2:(r0 + n) // 2, :], bf16)
        return pltpu.bitcast(w32[pl.ds(pl.multiple_of(r0 // 2, 8), n // 2), :], bf16)

    def rows(r0, n):
        return pl.ds(r0 if isinstance(r0, int) else pl.multiple_of(r0, 128), n)

    def W(ref, i, r0=None, n=None):
        if r0 is None:
            return pltpu.bitcast(ref[i], bf16)
        if not isinstance(r0, int):
            return pltpu.bitcast(ref[i, pl.ds(pl.multiple_of(r0 // 2, 8), n // 2), :], bf16)
        return pltpu.bitcast(ref[i, pl.ds(r0 // 2, n // 2), :], bf16)

    def glu_copies(c):
        c128 = pl.multiple_of(c * 128, 128) if not isinstance(c, int) else c * 128
        cps = [pltpu.make_async_copy(wg_hbm.at[:, pl.ds(c128, 128)], wall_v.at[rows((GO + c) * D, D)], semc.at[c]),
               pltpu.make_async_copy(wu_hbm.at[:, pl.ds(c128, 128)], wall_v.at[rows((UO + c) * D, D)], semc.at[c])]
        for n in range(KT):
            cps.append(pltpu.make_async_copy(wd_hbm.at[pl.ds(c128, 128), pl.ds(n * 128, 128)],
                                             wall_v.at[rows(DO + n * F + c128, 128)], semc.at[c]))
        return cps

    def x_copy(c):
        r0 = R + c * LNC
        if not isinstance(c, int):
            r0 = pl.multiple_of(r0, LNC)
        return pltpu.make_async_copy(x_hbm.at[pl.ds(r0, LNC)], x_v.at[pl.ds(r0, LNC)], semc.at[c])

    def raw_copies(m, i):
        src = (wq_hbm, wk_hbm, wv_hbm)[m].bitcast(u32)
        r0 = (i - m * (D // RAW)) * (RAW // 2)
        if not isinstance(i, int):
            r0 = pl.multiple_of(r0, RAW // 2)
        return [pltpu.make_async_copy(src.at[pl.ds(r0, RAW // 2), par, pl.ds(8 * g, 8), :],
                                      stage.at[i % NS, g, par], semr.at[i % NS])
                for g in range(2) for par in range(2)]

    def wo_copy(n):
        n128 = pl.multiple_of(n * 128, 128) if not isinstance(n, int) else n * 128
        return pltpu.make_async_copy(wo_hbm.at[:, pl.ds(n128, 128)], wo_v.at[n], semw.at[0])

    def start_group(c, lo, hi):
        assert hi <= lo or (lo // 8 == (hi - 1) // 8 or lo >= NRAW)

        def _when(cond_all, cond_none, cond, fn):
            if cond_all:
                fn()
            elif not cond_none:
                pl.when(cond())(fn)

        def g():
            for cp in glu_copies(c):
                cp.start()

        def r():
            for cp in raw_copies(lo // 8, c):
                cp.start()
        _when(hi <= FT, lo >= FT, lambda: c < FT, g)
        _when(hi <= NLN, lo >= NLN, lambda: c < NLN, lambda: x_copy(c).start())
        _when(hi <= NRAW, lo >= NRAW, lambda: c < NRAW, r)
        w0 = FT - KT + LA
        _when(lo >= w0 and hi <= w0 + KT, hi <= w0 or lo >= w0 + KT,
              lambda: jnp.logical_and(c >= w0, c < w0 + KT), lambda: wo_copy(c - w0).start())

    cx = pltpu.make_async_copy(x_hbm.at[pl.ds(0, R)], x_v.at[pl.ds(0, R)], sem0.at[0])
    cx.start()
    cm = pltpu.make_async_copy(mem0_hbm, mem_v, sem0.at[1])
    cm.start()
    for c in range(LA):
        start_group(c, c, c + 1)

    g_v[...] = jnp.zeros_like(g_v)
    cx.wait()

    def ln_body(i, _):
        r = pl.multiple_of(i * PB, PB)
        xn_v[pl.ds(r, PB), :] = _ln(x_v[pl.ds(r, PB), :].astype(f32))
        return 0
    lax.fori_loop(0, R // PB, ln_body, 0)

    def pro_body(lo, hi, c, _):
        for cp in glu_copies(c):
            cp.wait()
        if hi <= NLN:
            x_copy(c).wait()
        elif lo < NLN:
            pl.when(c < NLN)(lambda: x_copy(c).wait())
        if hi <= NRAW:
            pltpu.make_async_copy(stage.at[c % NS], stage.at[c % NS], semr.at[c % NS]).wait()
        assert hi <= NRAW or lo >= NRAW
        start_group(c + LA, lo + LA, hi + LA)

        i = jnp.minimum(c, NRAW - 1)
        m = i // (D // RAW)
        d0 = pl.multiple_of((i % (D // RAW)) * (RAW // 2), 8)

        def relayout(hp, t):
            g, j = hp // 8, hp % 8
            A = stage.at[i % NS, g, 0].reshape(RAW // 2 * 8, DH)[pl.ds(t * 64 + j, 8, stride=8), :]
            B = stage.at[i % NS, g, 1].reshape(RAW // 2 * 8, DH)[pl.ds(t * 64 + j, 8, stride=8), :]
            lo = (A & jnp.uint32(0xFFFF)) | (B << 16)
            hi = (A >> 16) | (B & jnp.uint32(0xFFFF0000))
            base = (m * H + 2 * hp) * (D // 2) + d0 + t * 8
            w32[pl.ds(pl.multiple_of(base, 8), 8), :] = lo
            w32[pl.ds(pl.multiple_of(base + D // 2, 8), 8), :] = hi

        c128 = pl.multiple_of(c * 128, 128)
        nb = R // PB
        hps = [(hp, t) for hp in range(H // 2) for t in range(RAW // 16)]
        nslots = nb * (2 * KT + KT) - 6
        cnt = [0]

        def fill():
            cnt[0] += 1
            tgt = min((len_hps * cnt[0]) // nslots, len_hps)
            if cnt[0] < nslots:
                tgt = (tgt // RG) * RG
            while len_hps - len(hps) < tgt:
                p_ = hps.pop(0)
                if lo < NRAW: relayout(*p_)
        len_hps = len(hps)

        def mm_k(xb_ref_rows, base):
            acc = None
            for kt in range(KT):
                t = _mm(xn_v[xb_ref_rows, kt * 128:(kt + 1) * 128], WS(base + kt * 128, 128))
                fill()
                acc = t if acc is None else acc + t
            return acc

        for b in range(nb):
            rs = slice(b * PB, (b + 1) * PB)
            gg = mm_k(rs, (GO + c) * D)
            uu = mm_k(rs, (UO + c) * D)
            hh = jax.nn.sigmoid(gg) * uu
            if b == 2:
                r = pl.multiple_of(R + jnp.minimum(c, NLN - 1) * LNC, LNC)
                xn_v[pl.ds(r, LNC), :] = _ln(x_v[pl.ds(r, LNC), :].astype(f32))
            for n in range(KT):
                g_v[b * PB:(b + 1) * PB, n * 128:(n + 1) * 128] += _mm(hh, wd32_tile(n, c128))
                fill()
        assert not hps
        return 0

    def wd32_tile(n, r0):
        return WS(DO + n * F + r0, 128)

    bounds = [0, 8 - LA, 16 - LA, 24 - LA, 24, FT]
    for lo, hi in zip(bounds[:-1], bounds[1:]):
        lax.fori_loop(lo, hi, functools.partial(pro_body, lo, hi), 0)
    cm.wait()
    pltpu.make_async_copy(wo_v, wo_v, semw.at[0]).wait()

    ri = lax.broadcasted_iota(jnp.int32, (L, L), 0)
    ci = lax.broadcasted_iota(jnp.int32, (L, L), 1)
    mask = (ri < M) | (ri >= ci)
    scale = DH ** -0.5

    def epilogue_compute(e):
        r0 = pl.multiple_of(e * SEG, SEG) if not isinstance(e, int) else e * SEG
        ga = g_v[pl.ds(r0, SEG), :]
        gl = ga * jax.nn.sigmoid(ga)
        res = x_v[pl.ds(r0, SEG), :].astype(f32) + s_v[pl.ds(r0, SEG), :] * gl
        o_v[pl.ds(r0, SEG), :] = res.astype(bf16)

    def epilogue_store(e):
        r0 = pl.multiple_of(e * SEG, SEG) if not isinstance(e, int) else e * SEG
        pltpu.make_async_copy(o_v.at[pl.ds(r0, SEG)], out_hbm.at[pl.ds(r0, SEG)], semo.at[0]).start()

    s_v[0:SEG, :] = jnp.zeros((SEG, D), f32)

    def step(s, mem):
        r0 = pl.multiple_of(s * SEG, SEG)
        h = jnp.concatenate([mem, xn_v[pl.ds(r0, SEG), :]], axis=0)
        qkv, scs, os_ = {}, {}, {}
        sb = s % CPB
        b0 = pl.multiple_of(R + (s // CPB) * RB, 8)
        xb = xn_v[pl.ds(b0, RB), :]
        hs = []

        def glu_gu(j):
            g = _mm(xb, WS((GO + sb * FC + j) * D, D))
            u = _mm(xb, WS((UO + sb * FC + j) * D, D))
            hs.append(jax.nn.sigmoid(g) * u)

        for i in range(H + LAG2):
            if i < H:
                q = _mm(h, WS(i * D, D))
                k = _mm(h, WS((H + i) * D, D)).astype(bf16)
                v = _mm(h, WS((2 * H + i) * D, D)).astype(bf16)
                qkv[i] = (q, k, v)
            else:
                glu_gu(i - H)
            if i == EPI_AT:
                epilogue_compute(jnp.maximum(s - ELAG, 0))
            j = i - LAG1
            if 0 <= j < H:
                q, k, v = qkv[j]
                sc = _mm_nt(q, k) * scale
                sc = jnp.where(mask, sc, -1e9)
                mx = jnp.max(sc, axis=-1, keepdims=True)
                e = jnp.exp(sc - mx)
                scs[j] = e / jnp.sum(e, axis=-1, keepdims=True)
            j = i - LAG2
            if 0 <= j < H:
                os_[j] = _mm(scs[j], qkv[j][2])
        for j in range(LAG2, FC):
            glu_gu(j)
        hh = jnp.concatenate(hs, axis=1)

        cols = []
        for n in range(KT):
            acc = None
            for hd in range(H):
                t = _mm(os_[hd], W(wo32, n, hd * 128, 128))
                acc = t if acc is None else acc + t
            cols.append(acc)
        o = jnp.concatenate(cols, axis=1)
        mem_next = o[:M].astype(bf16).astype(f32)
        s_v[pl.ds(r0, SEG), :] = o[M:]

        f0 = sb * (FC * 128)
        for n in range(KT):
            g_v[pl.ds(b0, RB), n * 128:(n + 1) * 128] += _mm(hh, WS(DO + n * F + f0, FC * 128))

        pl.when(s >= ELAG)(lambda: epilogue_store(s - ELAG))
        return mem_next

    lax.fori_loop(0, NSEG, step, mem_v[...].astype(f32))
    for e in range(NSEG - ELAG, NSEG):
        epilogue_compute(e)
        epilogue_store(e)
    pltpu.make_async_copy(o_v, out_hbm, semo.at[0]).wait()


@jax.jit
def pallas_recurrent_scan__memory_aug_recurrent_mem_tr__glu_gated_glu__prompt_kernel(
        A_x, A_mem0, A_Wq, A_Wk, A_Wv, A_Wo, A_seg_len, B_x, B_w_gate, B_w_up, B_w_down):
    x = A_x.reshape(S, D)
    mem0 = A_mem0.reshape(M, D)
    wq = A_Wq.reshape(D // 2, 2, H, DH)
    wk = A_Wk.reshape(D // 2, 2, H, DH)
    wv = A_Wv.reshape(D // 2, 2, H, DH)
    wo = A_Wo.reshape(H * DH, D)
    hbm = pl.BlockSpec(memory_space=pltpu.HBM)
    out = pl.pallas_call(
        _kernel,
        out_shape=jax.ShapeDtypeStruct((S, D), bf16),
        in_specs=[hbm] * 9,
        out_specs=hbm,
        scratch_shapes=[
            pltpu.VMEM((S, D), bf16),
            pltpu.VMEM((S, D), f32),
            pltpu.VMEM((M, D), bf16),
            pltpu.VMEM(((3 * H + 2 * FT) * D + KT * F, 128), bf16),
            pltpu.VMEM((KT, H * DH, 128), bf16),
            pltpu.VMEM((S, D), f32),
            pltpu.VMEM((S, D), f32),
            pltpu.VMEM((S, D), bf16),
            pltpu.VMEM((NS, 2, 2, RAW // 2, 8, DH), u32),
            pltpu.SemaphoreType.DMA((2,)),
            pltpu.SemaphoreType.DMA((FT,)),
            pltpu.SemaphoreType.DMA((NS,)),
            pltpu.SemaphoreType.DMA((1,)),
            pltpu.SemaphoreType.DMA((1,)),
        ],
        compiler_params=pltpu.CompilerParams(vmem_limit_bytes=120 * 2**20, disable_bounds_checks=True),
    )(x, mem0, wq, wk, wv, wo, B_w_gate, B_w_up, B_w_down)
    return out.reshape(1, S, D)
```

```python
import functools
import jax
import jax.numpy as jnp
from jax import lax
from jax.experimental import pallas as pl
from jax.experimental.pallas import tpu as pltpu

S, D, H, DH, M, SEG, F = 2048, 1024, 32, 128, 8, 32, 3584
L = M + SEG
NSEG = S // SEG
KT = D // 128
FT = F // 128
CPB = 4
FC = FT // CPB
RB = 88
R = S - (NSEG // CPB) * RB
PB = 128
LNC = 64
NLN = (S - R) // LNC
RAW = 128
NRAW = 3 * D // RAW
LA = 3
NS = 4
ELAG = 4
LAG1, LAG2 = 1, 3
EPI_AT = 8

RG = 8

f32 = jnp.float32
bf16 = jnp.bfloat16
u32 = jnp.uint32


def _mm(a, b):
    return lax.dot_general(a, b, (((1,), (0,)), ((), ())), preferred_element_type=f32)


def _mm_nt(a, b):
    return lax.dot_general(a, b, (((1,), (1,)), ((), ())), preferred_element_type=f32)


def _sig(t):
    return 0.5 * jnp.tanh(0.5 * t) + 0.5


def _ln(xx):
    m = jnp.mean(xx, axis=-1, keepdims=True)
    xc = xx - m
    v = jnp.mean(xc * xc, axis=-1, keepdims=True)
    return xc / jnp.sqrt(v + 1e-5)


def _kernel(x_hbm, mem0_hbm, wq_hbm, wk_hbm, wv_hbm, wo_hbm, wg_hbm, wu_hbm, wd_hbm,
            out_hbm,
            x_v, xn_v, mem_v, wall_v, wo_v,
            g_v, s_v, o_v, stage, sem0, semc, semr, semo, semw):
    w32, wo32 = wall_v.bitcast(u32), wo_v.bitcast(u32)
    GO, UO = 3 * H, 3 * H + FT
    DO = (3 * H + 2 * FT) * D

    def WS(r0, n):
        if isinstance(r0, int):
            return pltpu.bitcast(w32[r0 // 2:(r0 + n) // 2, :], bf16)
        return pltpu.bitcast(w32[pl.ds(pl.multiple_of(r0 // 2, 8), n // 2), :], bf16)

    def rows(r0, n):
        return pl.ds(r0 if isinstance(r0, int) else pl.multiple_of(r0, 128), n)

    def W(ref, i, r0=None, n=None):
        if r0 is None:
            return pltpu.bitcast(ref[i], bf16)
        if not isinstance(r0, int):
            return pltpu.bitcast(ref[i, pl.ds(pl.multiple_of(r0 // 2, 8), n // 2), :], bf16)
        return pltpu.bitcast(ref[i, pl.ds(r0 // 2, n // 2), :], bf16)

    def glu_copies(c):
        c128 = pl.multiple_of(c * 128, 128) if not isinstance(c, int) else c * 128
        cps = [pltpu.make_async_copy(wg_hbm.at[:, pl.ds(c128, 128)], wall_v.at[rows((GO + c) * D, D)], semc.at[c]),
               pltpu.make_async_copy(wu_hbm.at[:, pl.ds(c128, 128)], wall_v.at[rows((UO + c) * D, D)], semc.at[c])]
        for n in range(KT):
            cps.append(pltpu.make_async_copy(wd_hbm.at[pl.ds(c128, 128), pl.ds(n * 128, 128)],
                                             wall_v.at[rows(DO + n * F + c128, 128)], semc.at[c]))
        return cps

    def x_copy(c):
        r0 = R + c * LNC
        if not isinstance(c, int):
            r0 = pl.multiple_of(r0, LNC)
        return pltpu.make_async_copy(x_hbm.at[pl.ds(r0, LNC)], x_v.at[pl.ds(r0, LNC)], semc.at[c])

    def raw_copies(m, i):
        src = (wq_hbm, wk_hbm, wv_hbm)[m].bitcast(u32)
        r0 = (i - m * (D // RAW)) * (RAW // 2)
        if not isinstance(i, int):
            r0 = pl.multiple_of(r0, RAW // 2)
        return [pltpu.make_async_copy(src.at[pl.ds(r0, RAW // 2), par, pl.ds(8 * g, 8), :],
                                      stage.at[i % NS, g, par], semr.at[i % NS])
                for g in range(2) for par in range(2)]

    def wo_copy(n):
        n128 = pl.multiple_of(n * 128, 128) if not isinstance(n, int) else n * 128
        return pltpu.make_async_copy(wo_hbm.at[:, pl.ds(n128, 128)], wo_v.at[n], semw.at[0])

    def start_group(c, lo, hi):
        assert hi <= lo or (lo // 8 == (hi - 1) // 8 or lo >= NRAW)

        def _when(cond_all, cond_none, cond, fn):
            if cond_all:
                fn()
            elif not cond_none:
                pl.when(cond())(fn)

        def g():
            for cp in glu_copies(c):
                cp.start()

        def r():
            for cp in raw_copies(lo // 8, c):
                cp.start()
        _when(hi <= FT, lo >= FT, lambda: c < FT, g)
        _when(hi <= NLN, lo >= NLN, lambda: c < NLN, lambda: x_copy(c).start())
        _when(hi <= NRAW, lo >= NRAW, lambda: c < NRAW, r)
        w0 = FT - KT + LA
        _when(lo >= w0 and hi <= w0 + KT, hi <= w0 or lo >= w0 + KT,
              lambda: jnp.logical_and(c >= w0, c < w0 + KT), lambda: wo_copy(c - w0).start())

    cx = pltpu.make_async_copy(x_hbm.at[pl.ds(0, R)], x_v.at[pl.ds(0, R)], sem0.at[0])
    cx.start()
    cm = pltpu.make_async_copy(mem0_hbm, mem_v, sem0.at[1])
    cm.start()
    for c in range(LA):
        start_group(c, c, c + 1)

    g_v[...] = jnp.zeros_like(g_v)
    cx.wait()

    def ln_body(i, _):
        r = pl.multiple_of(i * PB, PB)
        xn_v[pl.ds(r, PB), :] = _ln(x_v[pl.ds(r, PB), :].astype(f32))
        return 0
    lax.fori_loop(0, R // PB, ln_body, 0)

    def pro_body(lo, hi, c, _):
        for cp in glu_copies(c):
            cp.wait()
        if hi <= NLN:
            x_copy(c).wait()
        elif lo < NLN:
            pl.when(c < NLN)(lambda: x_copy(c).wait())
        if hi <= NRAW:
            pltpu.make_async_copy(stage.at[c % NS], stage.at[c % NS], semr.at[c % NS]).wait()
        assert hi <= NRAW or lo >= NRAW
        start_group(c + LA, lo + LA, hi + LA)

        i = jnp.minimum(c, NRAW - 1)
        m = i // (D // RAW)
        d0 = pl.multiple_of((i % (D // RAW)) * (RAW // 2), 8)

        def relayout(hp, t):
            g, j = hp // 8, hp % 8
            A = stage.at[i % NS, g, 0].reshape(RAW // 2 * 8, DH)[pl.ds(t * 64 + j, 8, stride=8), :]
            B = stage.at[i % NS, g, 1].reshape(RAW // 2 * 8, DH)[pl.ds(t * 64 + j, 8, stride=8), :]
            lo = (A & jnp.uint32(0xFFFF)) | (B << 16)
            hi = (A >> 16) | (B & jnp.uint32(0xFFFF0000))
            base = (m * H + 2 * hp) * (D // 2) + d0 + t * 8
            w32[pl.ds(pl.multiple_of(base, 8), 8), :] = lo
            w32[pl.ds(pl.multiple_of(base + D // 2, 8), 8), :] = hi

        c128 = pl.multiple_of(c * 128, 128)
        nb = R // PB
        hps = [(hp, t) for hp in range(H // 2) for t in range(RAW // 16)]
        nslots = nb * (2 * KT + KT) - 6
        cnt = [0]

        def fill():
            cnt[0] += 1
            tgt = min((len_hps * cnt[0]) // nslots, len_hps)
            if cnt[0] < nslots:
                tgt = (tgt // RG) * RG
            while len_hps - len(hps) < tgt:
                p_ = hps.pop(0)
                if lo < NRAW: relayout(*p_)
        len_hps = len(hps)

        def mm_k(xb_ref_rows, base):
            acc = None
            for kt in range(KT):
                t = _mm(xn_v[xb_ref_rows, kt * 128:(kt + 1) * 128], WS(base + kt * 128, 128))
                fill()
                acc = t if acc is None else acc + t
            return acc

        for b in range(nb):
            rs = slice(b * PB, (b + 1) * PB)
            gg = mm_k(rs, (GO + c) * D)
            uu = mm_k(rs, (UO + c) * D)
            hh = _sig(gg) * uu
            if b == 2:
                r = pl.multiple_of(R + jnp.minimum(c, NLN - 1) * LNC, LNC)
                xn_v[pl.ds(r, LNC), :] = _ln(x_v[pl.ds(r, LNC), :].astype(f32))
            for n in range(KT):
                g_v[b * PB:(b + 1) * PB, n * 128:(n + 1) * 128] += _mm(hh, wd32_tile(n, c128))
                fill()
        assert not hps
        return 0

    def wd32_tile(n, r0):
        return WS(DO + n * F + r0, 128)

    bounds = [0, 8 - LA, 16 - LA, 24 - LA, 24, FT]
    for lo, hi in zip(bounds[:-1], bounds[1:]):
        lax.fori_loop(lo, hi, functools.partial(pro_body, lo, hi), 0)
    cm.wait()
    pltpu.make_async_copy(wo_v, wo_v, semw.at[0]).wait()

    ri = lax.broadcasted_iota(jnp.int32, (L, L), 0)
    ci = lax.broadcasted_iota(jnp.int32, (L, L), 1)
    mask = (ri < M) | (ri >= ci)
    scale = DH ** -0.5

    def epilogue_compute(e):
        r0 = pl.multiple_of(e * SEG, SEG) if not isinstance(e, int) else e * SEG
        ga = g_v[pl.ds(r0, SEG), :]
        gl = ga * _sig(ga)
        res = x_v[pl.ds(r0, SEG), :].astype(f32) + s_v[pl.ds(r0, SEG), :] * gl
        o_v[pl.ds(r0, SEG), :] = res.astype(bf16)

    def epilogue_store(e):
        r0 = pl.multiple_of(e * SEG, SEG) if not isinstance(e, int) else e * SEG
        pltpu.make_async_copy(o_v.at[pl.ds(r0, SEG)], out_hbm.at[pl.ds(r0, SEG)], semo.at[0]).start()

    s_v[0:SEG, :] = jnp.zeros((SEG, D), f32)

    def step(s, mem):
        r0 = pl.multiple_of(s * SEG, SEG)
        h = jnp.concatenate([mem, xn_v[pl.ds(r0, SEG), :]], axis=0)
        qkv, scs, os_ = {}, {}, {}
        sb = s % CPB
        b0 = pl.multiple_of(R + (s // CPB) * RB, 8)
        xb = xn_v[pl.ds(b0, RB), :]
        hs = []

        def glu_gu(j):
            g = _mm(xb, WS((GO + sb * FC + j) * D, D))
            u = _mm(xb, WS((UO + sb * FC + j) * D, D))
            hs.append(_sig(g) * u)

        for i in range(H + LAG2):
            if i < H:
                q = _mm(h, WS(i * D, D))
                k = _mm(h, WS((H + i) * D, D)).astype(bf16)
                v = _mm(h, WS((2 * H + i) * D, D)).astype(bf16)
                qkv[i] = (q, k, v)
            else:
                glu_gu(i - H)
            if i == EPI_AT:
                epilogue_compute(jnp.maximum(s - ELAG, 0))
            j = i - LAG1
            if 0 <= j < H:
                q, k, v = qkv[j]
                sc = _mm_nt(q, k) * scale
                sc = jnp.where(mask, sc, -1e9)
                mx = jnp.max(sc, axis=-1, keepdims=True)
                e = jnp.exp(sc - mx)
                scs[j] = e / jnp.sum(e, axis=-1, keepdims=True)
            j = i - LAG2
            if 0 <= j < H:
                os_[j] = _mm(scs[j], qkv[j][2])
        for j in range(LAG2, FC):
            glu_gu(j)
        hh = jnp.concatenate(hs, axis=1)

        cols = []
        for n in range(KT):
            acc = None
            for hd in range(H):
                t = _mm(os_[hd], W(wo32, n, hd * 128, 128))
                acc = t if acc is None else acc + t
            cols.append(acc)
        o = jnp.concatenate(cols, axis=1)
        mem_next = o[:M].astype(bf16).astype(f32)
        s_v[pl.ds(r0, SEG), :] = o[M:]

        f0 = sb * (FC * 128)
        for n in range(KT):
            g_v[pl.ds(b0, RB), n * 128:(n + 1) * 128] += _mm(hh, WS(DO + n * F + f0, FC * 128))

        pl.when(s >= ELAG)(lambda: epilogue_store(s - ELAG))
        return mem_next

    lax.fori_loop(0, NSEG, step, mem_v[...].astype(f32))
    for e in range(NSEG - ELAG, NSEG):
        epilogue_compute(e)
        epilogue_store(e)
    pltpu.make_async_copy(o_v, out_hbm, semo.at[0]).wait()


@jax.jit
def pallas_recurrent_scan__memory_aug_recurrent_mem_tr__glu_gated_glu__prompt_kernel(
        A_x, A_mem0, A_Wq, A_Wk, A_Wv, A_Wo, A_seg_len, B_x, B_w_gate, B_w_up, B_w_down):
    x = A_x.reshape(S, D)
    mem0 = A_mem0.reshape(M, D)
    wq = A_Wq.reshape(D // 2, 2, H, DH)
    wk = A_Wk.reshape(D // 2, 2, H, DH)
    wv = A_Wv.reshape(D // 2, 2, H, DH)
    wo = A_Wo.reshape(H * DH, D)
    hbm = pl.BlockSpec(memory_space=pltpu.HBM)
    out = pl.pallas_call(
        _kernel,
        out_shape=jax.ShapeDtypeStruct((S, D), bf16),
        in_specs=[hbm] * 9,
        out_specs=hbm,
        scratch_shapes=[
            pltpu.VMEM((S, D), bf16),
            pltpu.VMEM((S, D), f32),
            pltpu.VMEM((M, D), bf16),
            pltpu.VMEM(((3 * H + 2 * FT) * D + KT * F, 128), bf16),
            pltpu.VMEM((KT, H * DH, 128), bf16),
            pltpu.VMEM((S, D), f32),
            pltpu.VMEM((S, D), f32),
            pltpu.VMEM((S, D), bf16),
            pltpu.VMEM((NS, 2, 2, RAW // 2, 8, DH), u32),
            pltpu.SemaphoreType.DMA((2,)),
            pltpu.SemaphoreType.DMA((FT,)),
            pltpu.SemaphoreType.DMA((NS,)),
            pltpu.SemaphoreType.DMA((1,)),
            pltpu.SemaphoreType.DMA((1,)),
        ],
        compiler_params=pltpu.CompilerParams(vmem_limit_bytes=120 * 2**20, disable_bounds_checks=True),
    )(x, mem0, wq, wk, wv, wo, B_w_gate, B_w_up, B_w_down)
    return out.reshape(1, S, D)
```

```python
import functools
import jax
import jax.numpy as jnp
from jax import lax
from jax.experimental import pallas as pl
from jax.experimental.pallas import tpu as pltpu

S, D, H, DH, M, SEG, F = 2048, 1024, 32, 128, 8, 32, 3584
L = M + SEG
NSEG = S // SEG
KT = D // 128
FT = F // 128
CPB = 4
FC = FT // CPB
RB = 88
R = S - (NSEG // CPB) * RB
PB = 128
LNC = 64
NLN = (S - R) // LNC
RAW = 128
NRAW = 3 * D // RAW
LA = 3
NS = 4
ELAG = 4
LAG1, LAG2 = 1, 3
EPI_AT = 8
RG = 8

f32 = jnp.float32
bf16 = jnp.bfloat16
u32 = jnp.uint32


def _mm(a, b):
    return lax.dot_general(a, b, (((1,), (0,)), ((), ())), preferred_element_type=f32)


def _mm_nt(a, b):
    return lax.dot_general(a, b, (((1,), (1,)), ((), ())), preferred_element_type=f32)


def _sig(t):
    return 0.5 * jnp.tanh(0.5 * t) + 0.5


def _ln(xx):
    m = jnp.mean(xx, axis=-1, keepdims=True)
    xc = xx - m
    v = jnp.mean(xc * xc, axis=-1, keepdims=True)
    return xc / jnp.sqrt(v + 1e-5)


def _kernel(x_hbm, mem0_hbm, wq_hbm, wk_hbm, wv_hbm, wo_hbm, wg_hbm, wu_hbm, wd_hbm,
            out_hbm,
            x_v, xn_v, mem_v, wall_v, wo_v,
            g_v, s_v, o_v, stage, sem0, semc, semr, semo, semw):
    w32, wo32 = wall_v.bitcast(u32), wo_v.bitcast(u32)
    GO, UO = 3 * H, 3 * H + FT
    DO = (3 * H + 2 * FT) * D

    def WS(r0, n):
        if isinstance(r0, int):
            return pltpu.bitcast(w32[r0 // 2:(r0 + n) // 2, :], bf16)
        return pltpu.bitcast(w32[pl.ds(pl.multiple_of(r0 // 2, 8), n // 2), :], bf16)

    def rows(r0, n):
        return pl.ds(r0 if isinstance(r0, int) else pl.multiple_of(r0, 128), n)

    def W(ref, i, r0=None, n=None):
        if r0 is None:
            return pltpu.bitcast(ref[i], bf16)
        if not isinstance(r0, int):
            return pltpu.bitcast(ref[i, pl.ds(pl.multiple_of(r0 // 2, 8), n // 2), :], bf16)
        return pltpu.bitcast(ref[i, pl.ds(r0 // 2, n // 2), :], bf16)

    def glu_copies(c):
        c128 = pl.multiple_of(c * 128, 128) if not isinstance(c, int) else c * 128
        cps = [pltpu.make_async_copy(wg_hbm.at[:, pl.ds(c128, 128)], wall_v.at[rows((GO + c) * D, D)], semc.at[c]),
               pltpu.make_async_copy(wu_hbm.at[:, pl.ds(c128, 128)], wall_v.at[rows((UO + c) * D, D)], semc.at[c])]
        for n in range(KT):
            cps.append(pltpu.make_async_copy(wd_hbm.at[pl.ds(c128, 128), pl.ds(n * 128, 128)],
                                             wall_v.at[rows(DO + n * F + c128, 128)], semc.at[c]))
        return cps

    def x_copy(c):
        r0 = R + c * LNC
        if not isinstance(c, int):
            r0 = pl.multiple_of(r0, LNC)
        return pltpu.make_async_copy(x_hbm.at[pl.ds(r0, LNC)], x_v.at[pl.ds(r0, LNC)], semc.at[c])

    def raw_copies(m, i):
        src = (wq_hbm, wk_hbm, wv_hbm)[m].bitcast(u32)
        r0 = (i - m * (D // RAW)) * (RAW // 2)
        if not isinstance(i, int):
            r0 = pl.multiple_of(r0, RAW // 2)
        return [pltpu.make_async_copy(src.at[pl.ds(r0, RAW // 2), par, pl.ds(8 * g, 8), :],
                                      stage.at[i % NS, g, par], semr.at[i % NS])
                for g in range(2) for par in range(2)]

    def wo_copy(n):
        n128 = pl.multiple_of(n * 128, 128) if not isinstance(n, int) else n * 128
        return pltpu.make_async_copy(wo_hbm.at[:, pl.ds(n128, 128)], wo_v.at[n], semw.at[0])

    def start_group(c, lo, hi):
        assert hi <= lo or (lo // 8 == (hi - 1) // 8 or lo >= NRAW)

        def _when(cond_all, cond_none, cond, fn):
            if cond_all:
                fn()
            elif not cond_none:
                pl.when(cond())(fn)

        def g():
            for cp in glu_copies(c):
                cp.start()

        def r():
            for cp in raw_copies(lo // 8, c):
                cp.start()
        _when(hi <= FT, lo >= FT, lambda: c < FT, g)
        _when(hi <= NLN, lo >= NLN, lambda: c < NLN, lambda: x_copy(c).start())
        _when(hi <= NRAW, lo >= NRAW, lambda: c < NRAW, r)
        w0 = FT - KT + LA
        _when(lo >= w0 and hi <= w0 + KT, hi <= w0 or lo >= w0 + KT,
              lambda: jnp.logical_and(c >= w0, c < w0 + KT), lambda: wo_copy(c - w0).start())

    cx = pltpu.make_async_copy(x_hbm.at[pl.ds(0, R)], x_v.at[pl.ds(0, R)], sem0.at[0])
    cx.start()
    cm = pltpu.make_async_copy(mem0_hbm, mem_v, sem0.at[1])
    cm.start()
    for c in range(LA):
        start_group(c, c, c + 1)

    g_v[...] = jnp.zeros_like(g_v)
    cx.wait()

    def ln_body(i, _):
        r = pl.multiple_of(i * PB, PB)
        xn_v[pl.ds(r, PB), :] = _ln(x_v[pl.ds(r, PB), :].astype(f32))
        return 0
    lax.fori_loop(0, R // PB, ln_body, 0)

    def pro_body(lo, hi, c, _):
        for cp in glu_copies(c):
            cp.wait()
        if hi <= NLN:
            x_copy(c).wait()
        elif lo < NLN:
            pl.when(c < NLN)(lambda: x_copy(c).wait())
        if hi <= NRAW:
            pltpu.make_async_copy(stage.at[c % NS], stage.at[c % NS], semr.at[c % NS]).wait()
        assert hi <= NRAW or lo >= NRAW
        start_group(c + LA, lo + LA, hi + LA)

        i = jnp.minimum(c, NRAW - 1)
        m = i // (D // RAW)
        d0 = pl.multiple_of((i % (D // RAW)) * (RAW // 2), 8)

        def relayout(hp, t):
            g, j = hp // 8, hp % 8
            A = stage.at[i % NS, g, 0].reshape(RAW // 2 * 8, DH)[pl.ds(t * 64 + j, 8, stride=8), :]
            B = stage.at[i % NS, g, 1].reshape(RAW // 2 * 8, DH)[pl.ds(t * 64 + j, 8, stride=8), :]
            lo = (A & jnp.uint32(0xFFFF)) | (B << 16)
            hi = (A >> 16) | (B & jnp.uint32(0xFFFF0000))
            base = (m * H + 2 * hp) * (D // 2) + d0 + t * 8
            w32[pl.ds(pl.multiple_of(base, 8), 8), :] = lo
            w32[pl.ds(pl.multiple_of(base + D // 2, 8), 8), :] = hi

        c128 = pl.multiple_of(c * 128, 128)
        nb = R // PB
        hps = [(hp, t) for hp in range(H // 2) for t in range(RAW // 16)]
        nslots = nb * (2 * KT + KT) - 6
        cnt = [0]

        def fill():
            cnt[0] += 1
            tgt = min((len_hps * cnt[0]) // nslots, len_hps)
            if cnt[0] < nslots:
                tgt = (tgt // RG) * RG
            while len_hps - len(hps) < tgt:
                p_ = hps.pop(0)
                if lo < NRAW: relayout(*p_)
        len_hps = len(hps)

        def mm_k(xb_ref_rows, base):
            acc = None
            for kt in range(KT):
                t = _mm(xn_v[xb_ref_rows, kt * 128:(kt + 1) * 128], WS(base + kt * 128, 128))
                fill()
                acc = t if acc is None else acc + t
            return acc

        for b in range(nb):
            rs = slice(b * PB, (b + 1) * PB)
            gg = mm_k(rs, (GO + c) * D)
            uu = mm_k(rs, (UO + c) * D)
            hh = _sig(gg) * uu
            if b == 2:
                r = pl.multiple_of(R + jnp.minimum(c, NLN - 1) * LNC, LNC)
                xn_v[pl.ds(r, LNC), :] = _ln(x_v[pl.ds(r, LNC), :].astype(f32))
            for n in range(KT):
                g_v[b * PB:(b + 1) * PB, n * 128:(n + 1) * 128] += _mm(hh, wd32_tile(n, c128))
                fill()
        assert not hps
        return 0

    def wd32_tile(n, r0):
        return WS(DO + n * F + r0, 128)

    bounds = [0, 8 - LA, 16 - LA, 24 - LA, 24, FT]
    for lo, hi in zip(bounds[:-1], bounds[1:]):
        lax.fori_loop(lo, hi, functools.partial(pro_body, lo, hi), 0)
    cm.wait()
    pltpu.make_async_copy(wo_v, wo_v, semw.at[0]).wait()

    ri = lax.broadcasted_iota(jnp.int32, (L, L), 0)
    ci = lax.broadcasted_iota(jnp.int32, (L, L), 1)
    mask = (ri < M) | (ri >= ci)
    scale = DH ** -0.5

    def epilogue_compute(e):
        r0 = pl.multiple_of(e * SEG, SEG) if not isinstance(e, int) else e * SEG
        ga = g_v[pl.ds(r0, SEG), :]
        gl = ga * _sig(ga)
        res = x_v[pl.ds(r0, SEG), :].astype(f32) + s_v[pl.ds(r0, SEG), :] * gl
        o_v[pl.ds(r0, SEG), :] = res.astype(bf16)

    def epilogue_store(e):
        r0 = pl.multiple_of(e * SEG, SEG) if not isinstance(e, int) else e * SEG
        pltpu.make_async_copy(o_v.at[pl.ds(r0, SEG)], out_hbm.at[pl.ds(r0, SEG)], semo.at[0]).start()

    s_v[0:SEG, :] = jnp.zeros((SEG, D), f32)

    def step(t2, u, mem):
        s = t2 * 2 + u
        r0 = pl.multiple_of(s * SEG, SEG)
        h = jnp.concatenate([mem, xn_v[pl.ds(r0, SEG), :]], axis=0)
        qkv, scs, os_ = {}, {}, {}
        sb = s % CPB
        b0 = pl.multiple_of(R + (s // CPB) * RB, 8)
        xb = xn_v[pl.ds(b0, RB), :]
        hs = []

        def glu_gu(j):
            g = _mm(xb, WS((GO + sb * FC + j) * D, D))
            u = _mm(xb, WS((UO + sb * FC + j) * D, D))
            hs.append(_sig(g) * u)

        for i in range(H + LAG2):
            if i < H:
                q = _mm(h, WS(i * D, D))
                k = _mm(h, WS((H + i) * D, D)).astype(bf16)
                v = _mm(h, WS((2 * H + i) * D, D)).astype(bf16)
                qkv[i] = (q, k, v)
            else:
                glu_gu(i - H)
            if i == EPI_AT:
                epilogue_compute(jnp.maximum(s - ELAG, 0))
            j = i - LAG1
            if 0 <= j < H:
                q, k, v = qkv[j]
                sc = _mm_nt(q, k) * scale
                sc = jnp.where(mask, sc, -1e9)
                mx = jnp.max(sc, axis=-1, keepdims=True)
                e = jnp.exp(sc - mx)
                scs[j] = e / jnp.sum(e, axis=-1, keepdims=True)
            j = i - LAG2
            if 0 <= j < H:
                os_[j] = _mm(scs[j], qkv[j][2])
        for j in range(LAG2, FC):
            glu_gu(j)
        hh = jnp.concatenate(hs, axis=1)

        cols = []
        for n in range(KT):
            acc = None
            for hd in range(H):
                t = _mm(os_[hd], W(wo32, n, hd * 128, 128))
                acc = t if acc is None else acc + t
            cols.append(acc)
        o = jnp.concatenate(cols, axis=1)
        mem_next = o[:M].astype(bf16).astype(f32)
        s_v[pl.ds(r0, SEG), :] = o[M:]

        f0 = sb * (FC * 128)
        for n in range(KT):
            g_v[pl.ds(b0, RB), n * 128:(n + 1) * 128] += _mm(hh, WS(DO + n * F + f0, FC * 128))

        return mem_next

    def pair(t2, mem):
        for u in range(2):
            mem = step(t2, u, mem)

        @pl.when(t2 >= ELAG // 2)
        def _():
            r0 = pl.multiple_of((t2 - ELAG // 2) * (2 * SEG), 2 * SEG)
            pltpu.make_async_copy(o_v.at[pl.ds(r0, 2 * SEG)], out_hbm.at[pl.ds(r0, 2 * SEG)], semo.at[0]).start()
        return mem

    lax.fori_loop(0, NSEG // 2, pair, mem_v[...].astype(f32))
    for e in range(NSEG - ELAG, NSEG):
        epilogue_compute(e)
        epilogue_store(e)
    pltpu.make_async_copy(o_v, out_hbm, semo.at[0]).wait()


@jax.jit
def pallas_recurrent_scan__memory_aug_recurrent_mem_tr__glu_gated_glu__prompt_kernel(
        A_x, A_mem0, A_Wq, A_Wk, A_Wv, A_Wo, A_seg_len, B_x, B_w_gate, B_w_up, B_w_down):
    x = A_x.reshape(S, D)
    mem0 = A_mem0.reshape(M, D)
    wq = A_Wq.reshape(D // 2, 2, H, DH)
    wk = A_Wk.reshape(D // 2, 2, H, DH)
    wv = A_Wv.reshape(D // 2, 2, H, DH)
    wo = A_Wo.reshape(H * DH, D)
    hbm = pl.BlockSpec(memory_space=pltpu.HBM)
    out = pl.pallas_call(
        _kernel,
        out_shape=jax.ShapeDtypeStruct((S, D), bf16),
        in_specs=[hbm] * 9,
        out_specs=hbm,
        scratch_shapes=[
            pltpu.VMEM((S, D), bf16),
            pltpu.VMEM((S, D), f32),
            pltpu.VMEM((M, D), bf16),
            pltpu.VMEM(((3 * H + 2 * FT) * D + KT * F, 128), bf16),
            pltpu.VMEM((KT, H * DH, 128), bf16),
            pltpu.VMEM((S, D), f32),
            pltpu.VMEM((S, D), f32),
            pltpu.VMEM((S, D), bf16),
            pltpu.VMEM((NS, 2, 2, RAW // 2, 8, DH), u32),
            pltpu.SemaphoreType.DMA((2,)),
            pltpu.SemaphoreType.DMA((FT,)),
            pltpu.SemaphoreType.DMA((NS,)),
            pltpu.SemaphoreType.DMA((1,)),
            pltpu.SemaphoreType.DMA((1,)),
        ],
        compiler_params=pltpu.CompilerParams(vmem_limit_bytes=120 * 2**20, disable_bounds_checks=True),
    )(x, mem0, wq, wk, wv, wo, B_w_gate, B_w_up, B_w_down)
    return out.reshape(1, S, D)
```
